```python
import os as _os
_os.environ.setdefault("JAX_PLATFORMS", "cpu")
import jax
import jax.numpy as jnp

def _softmax(x, axis=-1):
    return jax.nn.softmax(x, axis=axis)
def _gelu(x):
    return jax.nn.gelu(x, approximate=True)
def _silu(x):
    return jax.nn.silu(x)
def _sigmoid(x):
    return jax.nn.sigmoid(x)
def _layernorm(x, axis=-1, eps=1e-5):
    m = jnp.mean(x, axis=axis, keepdims=True)
    v = jnp.var(x, axis=axis, keepdims=True)
    return (x - m) / jnp.sqrt(v + eps)
def _scatter_add(tgt, idx, src, axis=0):
    return tgt.at[idx].add(src)
def _segment_sum(src, seg, n):
    return jax.ops.segment_sum(src, seg, n)
class _Rng:
    def __init__(self, key):
        self._k = key
    def _next(self):
        self._k, sub = jax.random.split(self._k)
        return sub
    def normal(self, shape):
        return jax.random.normal(self._next(), shape, dtype=jnp.bfloat16)
    def randint(self, lo, hi, shape):
        return jax.random.randint(self._next(), shape, lo, hi, dtype=jnp.int32)
    def uniform(self, shape, lo=0.0, hi=1.0):
        return jax.random.uniform(self._next(), shape, jnp.bfloat16, lo, hi)
    def permutation(self, n):
        return jax.random.permutation(self._next(), n)


kernel_name = 'standalone__detection_seg_fpn_lateral__vision'

def setup_inputs():
    _rng = _Rng(jax.random.key(int.from_bytes(__import__("os").urandom(4), "little")))
    _w = (lambda a: (lambda t: t.astype(jnp.bfloat16) if jnp.issubdtype(t.dtype, jnp.floating) else t)(jnp.asarray(a)))
    H = W = (256 // 2) * 2
    C = 384
    k = 1
    return {
        "c_fine": _w((lambda *s: _rng.normal(s) * 0.05)(1, H, W, C)),
        "p_coarse": _w((lambda *s: _rng.normal(s) * 0.05)(1, H // 2, W // 2, C)),
        "w_lat": _w((lambda *s: _rng.normal(s) * 0.05)(C, C)),
        "w_out": _w((lambda *s: _rng.normal(s) * 0.05)(k, k, C, C)),
    }

def reference(c_fine, p_coarse, w_lat, w_out):
    B, H, W, C = c_fine.shape
    k = 1
    lat = jnp.einsum("bhwc,cd->bhwd", c_fine, w_lat)
    up = jnp.repeat(jnp.repeat(p_coarse, 2, axis=1), 2, axis=2)
    m = lat + up
    pad = k // 2
    mp = jnp.pad(m, ((0, 0), (pad, pad), (pad, pad), (0, 0)))
    o = None
    for di in range(k):
        for dj in range(k):
            t = jnp.einsum("bhwc,cd->bhwd", mp[:, di:di + H, dj:dj + W, :], w_out[di, dj])
            o = t if o is None else o + t
    return o
```

```python
import functools

import jax
import jax.numpy as jnp
from jax import lax
import jax.experimental.pallas as pl
import jax.experimental.pallas.tpu as pltpu

_dot = functools.partial(jnp.dot, preferred_element_type=jnp.float32)


def _repeat_rows_2x(q):
    bits = pltpu.bitcast(q.astype(jnp.bfloat16).astype(jnp.float32), jnp.uint32)
    return pltpu.bitcast(bits | (bits >> 16), jnp.bfloat16).astype(jnp.float32)


@jax.jit
def pallas_standalone__detection_seg_fpn_lateral__vision_kernel(
    c_fine: jax.Array,
    p_coarse: jax.Array,
    w_lat: jax.Array,
    w_out: jax.Array,
):
    _, H, W, C = c_fine.shape
    A, B = H // 4, 4 * W
    bounds = (0, 1, 2, 4, 7, 11, 18, 29, 46, 64)
    astar, nb, na, burst, rate, tail = 39, 32, 8, 32, 8, 256
    nch = len(bounds) - 1
    per_group = B // nb
    total = (A // na) * per_group

    def kernel(c_hbm, p_hbm, w1_hbm, w2_hbm, o_hbm, cb, pb, ob, w1b, w2b, w12b, rsem, wsem):
        wc = [pltpu.make_async_copy(w1_hbm, w1b, wsem), pltpu.make_async_copy(w2_hbm, w2b, wsem)]

        def rd(j):
            a0, a1 = bounds[j], bounds[j + 1]
            s = pl.ds(a0, a1 - a0)
            d = [pltpu.make_async_copy(p_hbm.at[s], pb.at[s], rsem.at[j])]
            if j == nch - 1:
                s = pl.ds(a0, a1 - a0 - 1)
                d.append(pltpu.make_async_copy(c_hbm.at[s], cb.at[s], rsem.at[j]))
                s = pl.ds(0, B - tail)
                d.append(pltpu.make_async_copy(c_hbm.at[A - 1, s], cb.at[A - 1, s], rsem.at[j]))
            else:
                d.append(pltpu.make_async_copy(c_hbm.at[s], cb.at[s], rsem.at[j]))
            return d

        s = pl.ds(B - tail, tail)
        tl = pltpu.make_async_copy(c_hbm.at[A - 1, s], cb.at[A - 1, s], rsem.at[nch])
        for d in wc:
            d.start()
        for j in range(nch):
            for d in rd(j):
                d.start(priority=1)
        tl.start(priority=1)
        for d in wc:
            d.wait()
        w12b[...] = _dot(w1b[...], w2b[...]).astype(jnp.bfloat16)

        def wr(i, _):
            a0 = (i // per_group) * na
            b0 = pl.multiple_of((i % per_group) * nb, nb)
            sl = (pl.ds(a0, na), pl.ds(b0, nb))
            pltpu.make_async_copy(ob.at[sl], o_hbm.at[sl], wsem).start(priority=1)

        def body(a, nw):
            for j in range(nch):
                @pl.when(a == min(bounds[j], astar))
                def _():
                    for d in rd(j):
                        d.wait()
            hi = jnp.where(a >= astar, jnp.minimum((a // na) * per_group, burst + (a - astar) * rate), 0)
            lax.fori_loop(nw, hi, wr, None)

            @pl.when(a == A - 1)
            def _():
                tl.wait()

            for r in range(2):
                up = _repeat_rows_2x(_dot(pb[a, pl.ds(r * W // 2, W // 2), :], w2b[...]))
                for k in range(2):
                    s = pl.ds((2 * r + k) * W, W)
                    ob[a, s, :] = (_dot(cb[a, s, :], w12b[...]) + up).astype(jnp.bfloat16)
            return hi

        nw = lax.fori_loop(0, A, body, 0)
        lax.fori_loop(nw, total, wr, None)
        pltpu.make_async_copy(ob, o_hbm, wsem).wait()

    bf16 = jnp.bfloat16
    out = pl.pallas_call(
        kernel,
        in_specs=[pl.BlockSpec(memory_space=pl.ANY)] * 4,
        out_specs=pl.BlockSpec(memory_space=pl.ANY),
        out_shape=jax.ShapeDtypeStruct((A, B, C), bf16),
        scratch_shapes=[
            pltpu.VMEM((A, B, C), bf16),
            pltpu.VMEM((A, B // 4, C), bf16),
            pltpu.VMEM((A, B, C), bf16),
            pltpu.VMEM((C, C), bf16),
            pltpu.VMEM((C, C), bf16),
            pltpu.VMEM((C, C), bf16),
            pltpu.SemaphoreType.DMA((nch + 1,)),
            pltpu.SemaphoreType.DMA,
        ],
        compiler_params=pltpu.CompilerParams(vmem_limit_bytes=116 * 2**20),
    )(c_fine.reshape(A, B, C), p_coarse.reshape(A, B // 4, C), w_lat, w_out.reshape(C, C))
    return out.reshape(1, H, W, C)
```

```python
import functools

import jax
import jax.numpy as jnp
from jax import lax
import jax.experimental.pallas as pl
import jax.experimental.pallas.tpu as pltpu

_BAND_ROWS = 16
_STREAMS = 8
_STEP_PX = 64
_PIECE_PX = 32
_READ_BANDS = 2
_READS_PER_STEP = 2 * (_STEP_PX // _PIECE_PX) * (_STREAMS // _READ_BANDS)
_WRITES_PER_STEP = 2 * (_STEP_PX // _PIECE_PX)
_BULK_ROWS = 2
_READ_SLOTS = (1, 0, 1, 2, 1, 1, 1, 2, 1, 1, 1, 2, 1, 1, 1, 2, 1, 1, 1, 1, 1, 2)
_WRITE_BURST = 48
_WRITE_RATE = 8


def _dot(a, b):
    return jnp.dot(a, b, preferred_element_type=jnp.float32)


def _bits(x, lo, size):
    return (x >> (lo.bit_length() - 1)) & (size - 1)


def _repeat_rows_2x(q):
    word = pltpu.bitcast(q.astype(jnp.bfloat16).astype(jnp.float32), jnp.uint32)
    return pltpu.bitcast(word | (word >> 16), jnp.bfloat16).astype(jnp.float32)


def _kernel(c_hbm, p_hbm, w_lat_hbm, w_out_hbm, o_hbm, in_buf, out_buf, w_lat, w_out, w_fold, sem):
    bands, rows, width, chans = c_hbm.shape
    groups = bands // _STREAMS
    steps_per_pair = width // _STEP_PX
    steps_per_group = (rows // 2) * steps_per_pair
    num_steps = groups * steps_per_group
    coarse_px = _STEP_PX // 2
    steps_per_p_row = width // coarse_px
    pieces_per_row = width // _PIECE_PX

    trickle_steps = num_steps - (_BULK_ROWS // 2) * steps_per_pair
    num_reads = trickle_steps * _READS_PER_STEP
    num_writes = num_steps * _WRITES_PER_STEP
    reads_issued_per_step = sum(_READ_SLOTS)
    assert reads_issued_per_step >= _READS_PER_STEP
    switch_step = pl.cdiv(num_reads - _READS_PER_STEP, reads_issued_per_step)
    p_cuts = (0, 2, *range(steps_per_p_row, num_steps, steps_per_p_row), num_steps - 2, num_steps)
    num_p_chunks = len(p_cuts) - 1
    assert switch_step <= min(trickle_steps, p_cuts[-2])

    def first_band(step):
        return _bits(step, steps_per_group, groups) * _STREAMS

    def first_row(step):
        return _bits(step, steps_per_pair, rows // 2) * 2

    def first_px(step):
        return _bits(step, 1, steps_per_pair) * _STEP_PX

    def p_row(step):
        return _bits(step, steps_per_p_row, rows // 4)

    def p_px(step):
        return _bits(step, 1, steps_per_p_row) * coarse_px

    def start_write(i, carry=None):
        window = (
            pl.ds(_bits(i, pieces_per_row * rows, groups) * _STREAMS, _STREAMS),
            _bits(i, pieces_per_row, rows),
            pl.ds(pl.multiple_of(_bits(i, 1, pieces_per_row) * _PIECE_PX, _PIECE_PX), _PIECE_PX),
        )
        pltpu.make_async_copy(out_buf.at[window], o_hbm.at[window], sem).start()

    def read_and_compute(bulk_sems, step_sems):
        def start_read(i, carry=None):
            band_sets = _STREAMS // _READ_BANDS
            pieces = _STEP_PX // _PIECE_PX
            step = _bits(i, _READS_PER_STEP, num_steps)
            px = first_px(step) + _bits(i, band_sets, pieces) * _PIECE_PX
            window = (
                pl.ds(first_band(step) + _bits(i, 1, band_sets) * _READ_BANDS, _READ_BANDS),
                first_row(step) + _bits(i, band_sets * pieces, 2),
                pl.ds(pl.multiple_of(px, _PIECE_PX), _PIECE_PX),
            )
            pltpu.make_async_copy(c_hbm.at[window], in_buf.at[window], step_sems.at[step]).start()

        def p_copy(j):
            lo, hi = p_cuts[j], p_cuts[j + 1]
            band, px = pl.ds(first_band(lo), _STREAMS), pl.ds(p_px(lo), (hi - lo) * coarse_px)
            return pltpu.make_async_copy(
                p_hbm.at[band, p_row(lo), px],
                in_buf.at[band, rows + p_row(lo), px],
                bulk_sems.at[j],
            )

        window = (pl.ds(bands - _STREAMS, _STREAMS), pl.ds(rows - _BULK_ROWS, _BULK_ROWS))
        c_bulk = pltpu.make_async_copy(c_hbm.at[window], in_buf.at[window], bulk_sems.at[num_p_chunks])
        weights = (
            pltpu.make_async_copy(w_lat_hbm, w_lat, bulk_sems.at[num_p_chunks + 1]),
            pltpu.make_async_copy(w_out_hbm, w_out, bulk_sems.at[num_p_chunks + 2]),
        )

        for copy in weights:
            copy.start()
        for j in range(num_p_chunks):
            if j == num_p_chunks - 2:
                c_bulk.start(priority=1)
            p_copy(j).start(priority=1)
        lax.fori_loop(0, _READS_PER_STEP, start_read, None)
        for copy in weights:
            copy.wait()
        w_fold[...] = _dot(w_lat[...], w_out[...]).astype(w_fold.dtype)

        def step_body(step, writes_done):
            slots = iter(range(len(_READ_SLOTS)))

            def issue_reads():
                slot = next(slots)
                base = _READS_PER_STEP + step * reads_issued_per_step + sum(_READ_SLOTS[:slot])
                for n in range(_READ_SLOTS[slot]):
                    pl.when(base + n < num_reads)(functools.partial(start_read, base + n))

            issue_reads()
            for j in range(num_p_chunks):
                last = j == num_p_chunks - 1
                pl.when(step == (p_cuts[j] if last else min(p_cuts[j], switch_step)))(p_copy(j).wait)
            pl.when(step == switch_step)(c_bulk.wait)

            finished = (step - _bits(step, 1, steps_per_pair)) * _WRITES_PER_STEP
            budget = _WRITE_BURST + (step - switch_step) * _WRITE_RATE
            writes_due = jnp.where(step >= switch_step, jnp.minimum(finished, budget), 0)
            lax.fori_loop(writes_done, writes_due, start_write, None)

            band0, row0 = first_band(step), first_row(step)
            px = pl.ds(pl.multiple_of(first_px(step), _STEP_PX), _STEP_PX)
            coarse = pl.ds(pl.multiple_of(p_px(step), coarse_px), coarse_px)

            @pl.when(step < trickle_steps)
            def _():
                filled = in_buf.at[pl.ds(band0, _STREAMS), pl.ds(row0, 2), px]
                pltpu.make_async_copy(filled, filled, step_sems.at[step]).wait()

            for b in range(0, _STREAMS, 2):
                issue_reads()
                p = in_buf[pl.ds(band0 + b, 2), rows + p_row(step), coarse, :]
                up = _repeat_rows_2x(_dot(p.reshape(2 * coarse_px, chans), w_out[...]))
                for db in range(2):
                    for dr in range(2):
                        issue_reads()
                        at = (band0 + b + db, row0 + dr, px, slice(None))
                        out = _dot(in_buf[at], w_fold[...]) + up[db * _STEP_PX : (db + 1) * _STEP_PX]
                        out_buf[at] = out.astype(out_buf.dtype)
            issue_reads()
            assert next(slots, None) is None
            return writes_due

        writes_done = lax.fori_loop(0, num_steps, step_body, 0)
        lax.fori_loop(writes_done, num_writes, start_write, None)

    pl.run_scoped(
        read_and_compute,
        pltpu.SemaphoreType.DMA((num_p_chunks + 3,)),
        pltpu.SemaphoreType.DMA((trickle_steps,)),
    )
    pltpu.make_async_copy(out_buf, o_hbm, sem).wait()


@jax.jit
def pallas_standalone__detection_seg_fpn_lateral__vision_kernel(
    c_fine: jax.Array,
    p_coarse: jax.Array,
    w_lat: jax.Array,
    w_out: jax.Array,
):
    batch, height, width, chans = c_fine.shape
    assert (batch, height, width) == (1, 256, 256) and w_out.shape[:2] == (1, 1)
    bands, dtype = height // _BAND_ROWS, c_fine.dtype
    fine_shape = (bands, _BAND_ROWS, width, chans)
    coarse_shape = (bands, _BAND_ROWS // 4, width, chans)

    out = pl.pallas_call(
        _kernel,
        in_specs=[pl.BlockSpec(memory_space=pl.ANY)] * 4,
        out_specs=pl.BlockSpec(memory_space=pl.ANY),
        out_shape=jax.ShapeDtypeStruct(fine_shape, dtype),
        scratch_shapes=[
            pltpu.VMEM((bands, _BAND_ROWS + _BAND_ROWS // 4, width, chans), dtype),
            pltpu.VMEM(fine_shape, dtype),
            pltpu.VMEM((chans, chans), dtype),
            pltpu.VMEM((chans, chans), dtype),
            pltpu.VMEM((chans, chans), dtype),
            pltpu.SemaphoreType.DMA,
        ],
        compiler_params=pltpu.CompilerParams(
            vmem_limit_bytes=116 * 1024 * 1024,
            disable_bounds_checks=True,
        ),
    )(
        c_fine.reshape(fine_shape),
        p_coarse.reshape(coarse_shape),
        w_lat,
        w_out.reshape(chans, chans),
    )
    return out.reshape(c_fine.shape)
```

```python
import jax
import jax.numpy as jnp
from jax import lax
import jax.experimental.pallas as pl
import jax.experimental.pallas.tpu as pltpu

_BAND_ROWS = 16
_STREAMS = 8
_STEP_PX = 64
_PIECE_PX = 32
_READ_BANDS = 2
_READS_PER_STEP = 2 * (_STEP_PX // _PIECE_PX) * (_STREAMS // _READ_BANDS)
_WRITES_PER_STEP = 2 * (_STEP_PX // _PIECE_PX)
_BULK_ROWS = 2
_READ_SLOTS = (1, 0, 1, 2, 1, 1, 1, 2, 1, 1, 1, 2, 1, 1, 1, 2, 1, 1, 1, 1, 1, 2)
_HEAD_STEPS = 2
_TAIL_STEPS = 2
_WRITE_RATE = 7


def _dot(a, b):
    return jnp.dot(a, b, preferred_element_type=jnp.float32)


def _digit(x, unit, base):
    return (x >> (unit.bit_length() - 1)) & (base - 1)


def _repeat_rows_2x(q):
    word = pltpu.bitcast(q.astype(jnp.bfloat16).astype(jnp.float32), jnp.uint32)
    return pltpu.bitcast(word | (word >> 16), jnp.bfloat16).astype(jnp.float32)


def _kernel(c_hbm, p_hbm, w_lat_hbm, w_out_hbm, o_hbm, in_buf, out_buf, w_lat, w_out, w_fold, out_sem):
    bands, rows, width, chans = c_hbm.shape
    groups = bands // _STREAMS
    coarse_px = _STEP_PX // 2
    steps_per_pair = width // _STEP_PX
    steps_per_p_row = width // coarse_px
    steps_per_group = (rows // 2) * steps_per_pair
    num_steps = groups * steps_per_group

    trickle_steps = num_steps - (_BULK_ROWS // 2) * steps_per_pair
    num_reads = trickle_steps * _READS_PER_STEP
    read_rate = sum(_READ_SLOTS)
    switch_step = (num_reads - _READS_PER_STEP) // read_rate
    first_reads = num_reads - switch_step * read_rate
    assert read_rate >= _READS_PER_STEP
    p_cuts = (
        0,
        _HEAD_STEPS,
        *range(steps_per_p_row, num_steps, steps_per_p_row),
        num_steps - _TAIL_STEPS,
        num_steps,
    )
    num_p_chunks = len(p_cuts) - 1
    assert switch_step <= min(trickle_steps, p_cuts[-2])

    num_writes = num_steps * _WRITES_PER_STEP
    last_writes = steps_per_pair * _WRITES_PER_STEP
    first_writes = num_writes - last_writes - (num_steps - switch_step) * _WRITE_RATE
    assert all(
        0 < first_writes + (s + 1 - switch_step) * _WRITE_RATE <= (s - s % steps_per_pair) * _WRITES_PER_STEP
        for s in range(switch_step, num_steps)
    )

    def first_band(step):
        return _digit(step, steps_per_group, groups) * _STREAMS

    def first_row(step):
        return _digit(step, steps_per_pair, rows // 2) * 2

    def first_px(step):
        return _digit(step, 1, steps_per_pair) * _STEP_PX

    def p_row(step):
        return _digit(step, steps_per_p_row, rows // 4)

    def p_px(step):
        return _digit(step, 1, steps_per_p_row) * coarse_px

    def compute(step, issue_point=lambda: None):
        band0, row0 = first_band(step), first_row(step)
        px = pl.ds(pl.multiple_of(first_px(step), _STEP_PX), _STEP_PX)
        coarse = pl.ds(pl.multiple_of(p_px(step), coarse_px), coarse_px)
        for b in range(0, _STREAMS, 2):
            issue_point()
            p = in_buf[pl.ds(band0 + b, 2), rows + p_row(step), coarse, :]
            up = _repeat_rows_2x(_dot(p.reshape(2 * coarse_px, chans), w_out[...]))
            for db in range(2):
                for dr in range(2):
                    issue_point()
                    at = (band0 + b + db, row0 + dr, px, slice(None))
                    out = _dot(in_buf[at], w_fold[...]) + up[db * _STEP_PX : (db + 1) * _STEP_PX]
                    out_buf[at] = out.astype(out_buf.dtype)
        issue_point()

    def start_write(i, _=None):
        pieces = width // _PIECE_PX
        window = (
            pl.ds(_digit(i, pieces * rows, groups) * _STREAMS, _STREAMS),
            _digit(i, pieces, rows),
            pl.ds(pl.multiple_of(_digit(i, 1, pieces) * _PIECE_PX, _PIECE_PX), _PIECE_PX),
        )
        pltpu.make_async_copy(out_buf.at[window], o_hbm.at[window], out_sem).start()

    def read_phase(bulk_sems, step_sems):
        def start_read(i, _=None):
            band_sets = _STREAMS // _READ_BANDS
            pieces = _STEP_PX // _PIECE_PX
            step = _digit(i, _READS_PER_STEP, num_steps)
            px = first_px(step) + _digit(i, band_sets, pieces) * _PIECE_PX
            window = (
                pl.ds(first_band(step) + _digit(i, 1, band_sets) * _READ_BANDS, _READ_BANDS),
                first_row(step) + _digit(i, band_sets * pieces, 2),
                pl.ds(pl.multiple_of(px, _PIECE_PX), _PIECE_PX),
            )
            pltpu.make_async_copy(c_hbm.at[window], in_buf.at[window], step_sems.at[step]).start()

        def wait_reads(step, _=None):
            filled = in_buf.at[
                pl.ds(first_band(step), _STREAMS),
                pl.ds(first_row(step), 2),
                pl.ds(pl.multiple_of(first_px(step), _STEP_PX), _STEP_PX),
            ]
            pltpu.make_async_copy(filled, filled, step_sems.at[step]).wait()

        def p_copy(j):
            lo, hi = p_cuts[j], p_cuts[j + 1]
            band, px = pl.ds(first_band(lo), _STREAMS), pl.ds(p_px(lo), (hi - lo) * coarse_px)
            return pltpu.make_async_copy(
                p_hbm.at[band, p_row(lo), px],
                in_buf.at[band, rows + p_row(lo), px],
                bulk_sems.at[j],
            )

        window = (pl.ds(bands - _STREAMS, _STREAMS), pl.ds(rows - _BULK_ROWS, _BULK_ROWS))
        c_bulk = pltpu.make_async_copy(c_hbm.at[window], in_buf.at[window], bulk_sems.at[num_p_chunks])
        weights = (
            pltpu.make_async_copy(w_lat_hbm, w_lat, bulk_sems.at[num_p_chunks + 1]),
            pltpu.make_async_copy(w_out_hbm, w_out, bulk_sems.at[num_p_chunks + 2]),
        )
        *p_chunks, p_tail = [p_copy(j) for j in range(num_p_chunks)]

        for copy in (*weights, p_chunks[0]):
            copy.start()
        for copy in (*p_chunks[1:], c_bulk, p_tail):
            copy.start(priority=1)
        lax.fori_loop(0, first_reads, start_read, None)
        for copy in weights:
            copy.wait()
        w_fold[...] = _dot(w_lat[...], w_out[...]).astype(w_fold.dtype)

        def read_step(step, _):
            slots = iter(range(len(_READ_SLOTS)))

            def issue_reads():
                slot = next(slots)
                for n in range(_READ_SLOTS[slot]):
                    start_read(first_reads + step * read_rate + sum(_READ_SLOTS[:slot]) + n)

            issue_reads()
            for needed_at, copy in zip(p_cuts, p_chunks):
                if needed_at < switch_step:
                    pl.when(step == needed_at)(copy.wait)
            wait_reads(step)
            compute(step, issue_reads)
            assert next(slots, None) is None

        lax.fori_loop(0, switch_step, read_step, None)

        for needed_at, copy in zip(p_cuts, p_chunks):
            if needed_at >= switch_step:
                copy.wait()
        c_bulk.wait()
        lax.fori_loop(0, first_writes, start_write, None)
        p_tail.wait()
        lax.fori_loop(switch_step, trickle_steps, wait_reads, None)

    pl.run_scoped(
        read_phase,
        pltpu.SemaphoreType.DMA((num_p_chunks + 3,)),
        pltpu.SemaphoreType.DMA((trickle_steps,)),
    )

    def write_step(step, _):
        first = first_writes + (step - switch_step) * _WRITE_RATE
        for n in range(_WRITE_RATE):
            start_write(first + n)
        compute(step)

    lax.fori_loop(switch_step, num_steps, write_step, None)
    lax.fori_loop(num_writes - last_writes, num_writes, start_write, None)
    pltpu.make_async_copy(out_buf, o_hbm, out_sem).wait()


@jax.jit
def pallas_standalone__detection_seg_fpn_lateral__vision_kernel(
    c_fine: jax.Array,
    p_coarse: jax.Array,
    w_lat: jax.Array,
    w_out: jax.Array,
):
    batch, height, width, chans = c_fine.shape
    assert (batch, height, width) == (1, 256, 256) and w_out.shape[:2] == (1, 1)
    bands, dtype = height // _BAND_ROWS, c_fine.dtype
    fine_shape = (bands, _BAND_ROWS, width, chans)
    coarse_shape = (bands, _BAND_ROWS // 4, width, chans)

    out = pl.pallas_call(
        _kernel,
        in_specs=[pl.BlockSpec(memory_space=pl.ANY)] * 4,
        out_specs=pl.BlockSpec(memory_space=pl.ANY),
        out_shape=jax.ShapeDtypeStruct(fine_shape, dtype),
        scratch_shapes=[
            pltpu.VMEM((bands, _BAND_ROWS + _BAND_ROWS // 4, width, chans), dtype),
            pltpu.VMEM(fine_shape, dtype),
            pltpu.VMEM((chans, chans), dtype),
            pltpu.VMEM((chans, chans), dtype),
            pltpu.VMEM((chans, chans), dtype),
            pltpu.SemaphoreType.DMA,
        ],
        compiler_params=pltpu.CompilerParams(vmem_limit_bytes=116 * 1024 * 1024),
    )(
        c_fine.reshape(fine_shape),
        p_coarse.reshape(coarse_shape),
        w_lat,
        w_out.reshape(chans, chans),
    )
    return out.reshape(c_fine.shape)
```
